```python
import jax
import jax.numpy as jnp

def _softmax(x, axis=-1):
    return jax.nn.softmax(x, axis=axis)

def _gelu(x):
    return jax.nn.gelu(x, approximate=True)

def _silu(x):
    return jax.nn.silu(x)

def _sigmoid(x):
    return jax.nn.sigmoid(x)

def _layernorm(x, axis=-1, eps=1e-05):
    m = jnp.mean(x, axis=axis, keepdims=True)
    v = jnp.var(x, axis=axis, keepdims=True)
    return (x - m) / jnp.sqrt(v + eps)

def _scatter_add(tgt, idx, src, axis=0):
    return tgt.at[idx].add(src)

def _segment_sum(src, seg, n):
    return jax.ops.segment_sum(src, seg, n)

class _Rng:

    def __init__(self, key):
        self._k = key

    def _next(self):
        self._k, sub = jax.random.split(self._k)
        return sub

    def normal(self, shape):
        return jax.random.normal(self._next(), shape, dtype=jnp.bfloat16)

    def randint(self, lo, hi, shape):
        return jax.random.randint(self._next(), shape, lo, hi, dtype=jnp.int32)

    def uniform(self, shape, lo=0.0, hi=1.0):
        return jax.random.uniform(self._next(), shape, jnp.bfloat16, lo, hi)

    def permutation(self, n):
        return jax.random.permutation(self._next(), n)
kernel_name = 'adaLN_cond__compressed_kv_cla__mixer_s_mlp__decode'

def setup_inputs():
    _rng = _Rng(jax.random.key(int.from_bytes(__import__("os").urandom(4), "little")))
    _w = lambda a: (lambda t: t.astype(jnp.bfloat16) if jnp.issubdtype(t.dtype, jnp.floating) else t)(jnp.asarray(a))

    def _A_setup():
        B, H, Sq, Sk, D, M = (8, 32, 1, 4096, 128, 512)
        Dc = 4 * D
        return {'x': _w((lambda *s: _rng.normal(s) * 0.05)(B, Sq, M)), 'c_kv': _w((lambda *s: _rng.normal(s) * 0.05)(B, Sk, Dc)), 'w_q': _w((lambda *s: _rng.normal(s) * 0.05)(M, H, D) * M ** (-0.5)), 'w_uk': _w((lambda *s: _rng.normal(s) * 0.05)(Dc, H, D) * Dc ** (-0.5)), 'w_uv': _w((lambda *s: _rng.normal(s) * 0.05)(Dc, H, D) * Dc ** (-0.5)), 'w_o': _w((lambda *s: _rng.normal(s) * 0.05)(H, D, M) * (H * D) ** (-0.5))}
    _A_in = _A_setup()

    def _B_setup():
        B, S, D, F = (8, 1, 512, 1792)
        return {'x': _w((lambda *s: _rng.normal(s) * 0.05)(B, S, D)), 'w1': _w((lambda *s: _rng.normal(s) * 0.05)(D, D) * D ** (-0.5)), 'w2': _w((lambda *s: _rng.normal(s) * 0.05)(D, D) * D ** (-0.5)), 'w3': _w((lambda *s: _rng.normal(s) * 0.05)(D, F) * D ** (-0.5)), 'w4': _w((lambda *s: _rng.normal(s) * 0.05)(F, D) * F ** (-0.5))}
    _B_in = _B_setup()
    return {'A_x': _A_in['x'], 'A_c_kv': _A_in['c_kv'], 'A_w_q': _A_in['w_q'], 'A_w_uk': _A_in['w_uk'], 'A_w_uv': _A_in['w_uv'], 'A_w_o': _A_in['w_o'], 'B_x': _B_in['x'], 'B_w1': _B_in['w1'], 'B_w2': _B_in['w2'], 'B_w3': _B_in['w3'], 'B_w4': _B_in['w4'], 'c': _w((lambda *s: _rng.normal(s) * 0.05)(8, 512)), 'w_mod': _w((lambda *s: _rng.normal(s) * 0.05)(512, 6 * 512) * 512 ** (-0.5))}

def reference(A_x, A_c_kv, A_w_q, A_w_uk, A_w_uv, A_w_o, B_x, B_w1, B_w2, B_w3, B_w4, c, w_mod):

    def _A_ref(x, c_kv, w_q, w_uk, w_uv, w_o):
        B, Sq, M = (x.shape[0], x.shape[1], x.shape[2])
        Sk = c_kv.shape[1]
        H, D = (w_q.shape[1], w_q.shape[2])
        q = jnp.einsum('bqm,mhd->bhqd', x, w_q)
        k = jnp.einsum('bkc,chd->bhkd', c_kv, w_uk)
        v = jnp.einsum('bkc,chd->bhkd', c_kv, w_uv)
        scores = jnp.einsum('bhqd,bhkd->bhqk', q, k) * D ** (-0.5)
        off = Sk - Sq
        qi = jnp.arange(Sq)[:, None]
        kj = jnp.arange(Sk)[None, :]
        cmask = kj <= qi + off
        scores = jnp.where(cmask[None, None], scores, -1000000000.0)
        p = _softmax(scores, axis=-1)
        ctx = jnp.einsum('bhqk,bhkd->bhqd', p, v)
        return jnp.einsum('bhqd,hdm->bqm', ctx, w_o)

    def _B_ref(x, w1, w2, w3, w4):
        B, S, D = x.shape
        h = _gelu(_layernorm(x, axis=-1) @ w1)
        c = D // 4
        g0 = jnp.pad(h[:, :, 0 * c:1 * c], ((0, 0), (1, 0), (0, 0)))[:, :S, :]
        g1 = jnp.pad(h[:, :, 1 * c:2 * c], ((0, 0), (0, 1), (0, 0)))[:, 1:, :]
        g2 = jnp.pad(h[:, :, 2 * c:3 * c], ((0, 0), (2, 0), (0, 0)))[:, :S, :]
        g3 = jnp.pad(h[:, :, 3 * c:], ((0, 0), (0, 2), (0, 0)))[:, 2:, :]
        hs = jnp.concatenate([g0, g1, g2, g3], axis=-1) @ w2
        x1 = x + hs
        h2 = _gelu(_layernorm(x1, axis=-1) @ w3) @ w4
        return x1 + h2
    x = A_x
    mod = (_silu(c) @ w_mod).reshape(c.shape[0], 6, 1, -1)
    sa, ca, ga, sb, cb, gb = (mod[:, 0].copy(), mod[:, 1].copy(), mod[:, 2].copy(), mod[:, 3].copy(), mod[:, 4].copy(), mod[:, 5].copy())
    h = _layernorm(x, axis=-1) * (1 + ca) + sa
    x = x + ga * _A_ref(h, A_c_kv, A_w_q, A_w_uk, A_w_uv, A_w_o)
    h = _layernorm(x, axis=-1) * (1 + cb) + sb
    x = x + gb * _B_ref(h, B_w1, B_w2, B_w3, B_w4)
    return x
```

```python
import jax
import jax.numpy as jnp
import jax.experimental.pallas as pl
import jax.experimental.pallas.tpu as pltpu

_F32 = jnp.float32
_BF16 = jnp.bfloat16
_U32 = jnp.uint32
_NN = (((1,), (0,)), ((), ()))
_NT = (((1,), (1,)), ((), ()))
_LANES = 128


def _dot(a, b, dims=_NN):
    return jax.lax.dot_general(a, b, dims, preferred_element_type=_F32)


def _layernorm(x, eps=1e-5):
    m = jnp.mean(x, axis=-1, keepdims=True)
    d = x - m
    v = jnp.mean(d * d, axis=-1, keepdims=True)
    return d * jax.lax.rsqrt(v + eps)


def _head_pair(w32, j, rows, pairs):
    even = w32[pl.ds(j, rows // 2, stride=2 * pairs), :]
    odd = w32[pl.ds(j + pairs, rows // 2, stride=2 * pairs), :]
    lo = (even & _U32(0xFFFF)) | (odd << 16)
    hi = (even >> 16) | (odd & _U32(0xFFFF0000))
    return pltpu.bitcast(lo, _BF16), pltpu.bitcast(hi, _BF16)


def _make_kernel(B, Sk, M, Dc, H, D, F, wo_chunks, w4_chunks):
    P = H // 2
    scale = float(D) ** -0.5

    def kernel(x_hbm, kv_hbm, wq_hbm, wuk_hbm, wuv_hbm, wo_hbm, w3_hbm, w4_hbm, c_hbm, wmod_hbm,
               out_ref,
               x_v, kv_v, wq32, wuk32, wuv32, wo_v, w3_v, w4_v, c_v, wmod_v,
               q_s, qa_s, cc_s, ctx_s, sem, kv_sem):
        def whole(src, dst, k):
            return pltpu.make_async_copy(src, dst, sem.at[k])

        def rows(src, dst, lo, n, k):
            return pltpu.make_async_copy(src.at[pl.ds(lo, n)], dst.at[pl.ds(lo, n)], sem.at[k])

        def kv_copy(b):
            return pltpu.make_async_copy(kv_hbm.at[b], kv_v.at[b], kv_sem.at[b])

        cp_wmod = whole(wmod_hbm, wmod_v, 0)
        cp_c = whole(c_hbm, c_v, 1)
        cp_x = whole(x_hbm, x_v, 2)
        cp_wq = whole(wq_hbm, wq32.bitcast(_BF16), 3)
        cp_wuk = whole(wuk_hbm, wuk32.bitcast(_BF16), 4)
        cp_wuv = whole(wuv_hbm, wuv32.bitcast(_BF16), 5)
        cp_w3 = whole(w3_hbm, w3_v, 6)
        cp_wo = [rows(wo_hbm, wo_v, lo, n, 7 + i) for i, (lo, n) in enumerate(wo_chunks)]
        cp_w4 = [rows(w4_hbm, w4_v, lo, n, 7 + len(wo_chunks) + i)
                 for i, (lo, n) in enumerate(w4_chunks)]

        cp_wmod.start()
        cp_c.start()
        cp_x.start()
        cp_wq.start()
        cp_wuk.start()
        for b in range(B):
            kv_copy(b).start()
        cp_wuv.start()
        for cp in cp_wo:
            cp.start()
        cp_w3.start()
        for cp in cp_w4:
            cp.start()

        cp_c.wait()
        c = c_v[...].astype(_F32)
        sc = (c * jax.nn.sigmoid(c)).astype(_BF16)
        cp_x.wait()
        x = x_v[...].astype(_F32)
        xn = _layernorm(x)
        cp_wmod.wait()
        mod = _dot(sc, wmod_v[...])
        sa, ca, ga, sb, cb, gb = (mod[:, i * M:(i + 1) * M] for i in range(6))
        h = (xn * (1.0 + ca) + sa).astype(_BF16)

        cp_wq.wait()

        @pl.loop(0, P)
        def _(j):
            lo, hi = _head_pair(wq32, j, M, P)
            q2 = _dot(h, jnp.concatenate([lo, hi], axis=1))
            q_s[j] = q2

        cp_wuk.wait()

        @pl.loop(0, P)
        def _(j):
            q2 = q_s[j].astype(_BF16)
            for t, w in enumerate(_head_pair(wuk32, j, Dc, P)):
                qa = _dot(q2[:, t * D:(t + 1) * D], w, _NT)
                r = pl.multiple_of((2 * j + t) * B, B)
                for n in range(Dc // _LANES):
                    qa_s[n, pl.ds(r, B), :] = qa[:, n * _LANES:(n + 1) * _LANES]

        @pl.loop(0, B)
        def _(b):
            qa = jnp.concatenate(
                [qa_s[n, pl.ds(b, H, stride=B), :] for n in range(Dc // _LANES)], axis=1
            ).astype(_BF16)
            kv_copy(b).wait()
            kv = kv_v.at[b]
            s = _dot(qa, kv[...], _NT) * scale
            p = jnp.exp(s - jnp.max(s, axis=-1, keepdims=True))
            l = jnp.sum(p, axis=-1, keepdims=True)
            cc = _dot(p.astype(_BF16), kv[...]) / l
            r = pl.multiple_of(b * H, H)
            for n in range(Dc // _LANES):
                cc_s[n, pl.ds(r, H), :] = cc[:, n * _LANES:(n + 1) * _LANES]

        cp_wuv.wait()

        @pl.loop(0, P)
        def _(j):
            for t, w in enumerate(_head_pair(wuv32, j, Dc, P)):
                cc = jnp.concatenate(
                    [cc_s[n, pl.ds(2 * j + t, B, stride=H), :] for n in range(Dc // _LANES)],
                    axis=1,
                ).astype(_BF16)
                ctx_s[2 * j + t] = _dot(cc, w)

        att = jnp.zeros((B, M), _F32)
        for cp, (lo, n) in zip(cp_wo, wo_chunks):
            cp.wait()
            ctx = jnp.concatenate(
                [ctx_s[hh] for hh in range(lo // D, (lo + n) // D)], axis=1
            ).astype(_BF16)
            att = att + _dot(ctx, wo_v[pl.ds(lo, n), :])

        x = x + ga * att
        h2 = _layernorm(x) * (1.0 + cb) + sb
        hn = _layernorm(h2).astype(_BF16)

        cp_w3.wait()
        g = jax.nn.gelu(_dot(hn, w3_v[...]), approximate=True).astype(_BF16)
        acc = h2
        for cp, (lo, n) in zip(cp_w4, w4_chunks):
            cp.wait()
            acc = acc + _dot(g[:, lo:lo + n], w4_v[pl.ds(lo, n), :])
        out_ref[...] = (x + gb * acc).astype(out_ref.dtype)

    return kernel


@jax.jit
def pallas_adaLN_cond__compressed_kv_cla__mixer_s_mlp__decode_kernel(
    A_x: jax.Array,
    A_c_kv: jax.Array,
    A_w_q: jax.Array,
    A_w_uk: jax.Array,
    A_w_uv: jax.Array,
    A_w_o: jax.Array,
    B_x: jax.Array,
    B_w1: jax.Array,
    B_w2: jax.Array,
    B_w3: jax.Array,
    B_w4: jax.Array,
    c: jax.Array,
    w_mod: jax.Array,
):
    del B_x, B_w1, B_w2
    B, Sq, M = A_x.shape
    _, Sk, Dc = A_c_kv.shape
    _, H, D = A_w_q.shape
    F = B_w3.shape[1]
    assert Sq == 1 and D == _LANES and B == 8 and H % 16 == 0

    wo_chunks = [(0, H * D // 2), (H * D // 2, H * D // 2)]
    w4_chunks = [(0, F - 256), (F - 256, 256)]
    n_sem = 7 + len(wo_chunks) + len(w4_chunks)

    operands = (
        A_x.reshape(B, M),
        A_c_kv,
        A_w_q.reshape(M * H, D),
        A_w_uk.reshape(Dc * H, D),
        A_w_uv.reshape(Dc * H, D),
        A_w_o.reshape(H * D, M),
        B_w3,
        B_w4,
        c,
        w_mod,
    )
    out = pl.pallas_call(
        _make_kernel(B, Sk, M, Dc, H, D, F, wo_chunks, w4_chunks),
        out_shape=jax.ShapeDtypeStruct((B, M), A_x.dtype),
        in_specs=[pl.BlockSpec(memory_space=pl.ANY)] * len(operands),
        out_specs=pl.BlockSpec(memory_space=pltpu.VMEM),
        scratch_shapes=[
            pltpu.VMEM((a.shape[0] // 2, D), _U32) if i in (2, 3, 4) else pltpu.VMEM(a.shape, a.dtype)
            for i, a in enumerate(operands)] + [
            pltpu.VMEM((H // 2, B, 2 * D), _F32),
            pltpu.VMEM((Dc // _LANES, H * B, _LANES), _F32),
            pltpu.VMEM((Dc // _LANES, B * H, _LANES), _F32),
            pltpu.VMEM((H, B, D), _F32),
            pltpu.SemaphoreType.DMA((n_sem,)),
            pltpu.SemaphoreType.DMA((B,)),
        ],
        compiler_params=pltpu.CompilerParams(vmem_limit_bytes=100 * 2**20),
    )(*operands)
    return out.reshape(B, Sq, M)
```

```python
import jax
import jax.numpy as jnp
import jax.experimental.pallas as pl
import jax.experimental.pallas.tpu as pltpu

_F32 = jnp.float32
_BF16 = jnp.bfloat16
_U32 = jnp.uint32
_NN = (((1,), (0,)), ((), ()))
_NT = (((1,), (1,)), ((), ()))
_LANES = 128


def _dot(a, b, dims=_NN):
    return jax.lax.dot_general(a, b, dims, preferred_element_type=_F32)


def _layernorm(x, eps=1e-5):
    m = jnp.mean(x, axis=-1, keepdims=True)
    d = x - m
    v = jnp.mean(d * d, axis=-1, keepdims=True)
    return d * jax.lax.rsqrt(v + eps)


def _head_pair(w32, j, rows, pairs):
    even = w32[pl.ds(j, rows // 2, stride=2 * pairs), :]
    odd = w32[pl.ds(j + pairs, rows // 2, stride=2 * pairs), :]
    lo = (even & _U32(0xFFFF)) | (odd << 16)
    hi = (even >> 16) | (odd & _U32(0xFFFF0000))
    return pltpu.bitcast(lo, _BF16), pltpu.bitcast(hi, _BF16)


def _make_kernel(B, Sk, M, Dc, H, D, F, wo_chunks, w4_chunks):
    P = H // 2
    scale = float(D) ** -0.5

    def kernel(x_hbm, kv_hbm, wq_hbm, wuk_hbm, wuv_hbm, wo_hbm, w3_hbm, w4_hbm, c_hbm, wmod_hbm,
               out_ref,
               x_v, kv_v, wq32, wuk32, wuv32, wo_v, w3_v, w4_v, c_v, wmod_v,
               q_s, qa_s, cc_s, ctx_s, sem, kv_sem):
        def whole(src, dst, k):
            return pltpu.make_async_copy(src, dst, sem.at[k])

        def rows(src, dst, lo, n, k):
            return pltpu.make_async_copy(src.at[pl.ds(lo, n)], dst.at[pl.ds(lo, n)], sem.at[k])

        def kv_copy(b):
            return pltpu.make_async_copy(kv_hbm.at[b], kv_v.at[b], kv_sem.at[b])

        cp_wmod = whole(wmod_hbm, wmod_v, 0)
        cp_c = whole(c_hbm, c_v, 1)
        cp_x = whole(x_hbm, x_v, 2)
        cp_wq = whole(wq_hbm, wq32.bitcast(_BF16), 3)
        cp_wuk = whole(wuk_hbm, wuk32.bitcast(_BF16), 4)
        cp_wuv = whole(wuv_hbm, wuv32.bitcast(_BF16), 5)
        cp_w3 = whole(w3_hbm, w3_v, 6)
        cp_wo = [rows(wo_hbm, wo_v, lo, n, 7 + i) for i, (lo, n) in enumerate(wo_chunks)]
        cp_w4 = [rows(w4_hbm, w4_v, lo, n, 7 + len(wo_chunks) + i)
                 for i, (lo, n) in enumerate(w4_chunks)]

        AHEAD = 3
        cp_wmod.start()
        cp_c.start()
        cp_x.start()
        cp_wq.start()
        cp_wuk.start()
        for b in range(AHEAD):
            kv_copy(b).start()

        cp_c.wait()
        c = c_v[...].astype(_F32)
        sc = (c * jax.nn.sigmoid(c)).astype(_BF16)
        cp_x.wait()
        x = x_v[...].astype(_F32)
        xn = _layernorm(x)
        cp_wmod.wait()
        mod = _dot(sc, wmod_v[...])
        sa, ca, ga, sb, cb, gb = (mod[:, i * M:(i + 1) * M] for i in range(6))
        h = (xn * (1.0 + ca) + sa).astype(_BF16)

        cp_wq.wait()

        @pl.loop(0, P)
        def _(j):
            lo, hi = _head_pair(wq32, j, M, P)
            q2 = _dot(h, jnp.concatenate([lo, hi], axis=1))
            q_s[j] = q2

        cp_wuk.wait()

        @pl.loop(0, P)
        def _(j):
            q2 = q_s[j].astype(_BF16)
            for t, w in enumerate(_head_pair(wuk32, j, Dc, P)):
                qa = _dot(q2[:, t * D:(t + 1) * D], w, _NT)
                r = pl.multiple_of((2 * j + t) * B, B)
                for n in range(Dc // _LANES):
                    qa_s[n, pl.ds(r, B), :] = qa[:, n * _LANES:(n + 1) * _LANES]

        @pl.loop(0, B)
        def _(b):
            qa = jnp.concatenate(
                [qa_s[n, pl.ds(b, H, stride=B), :] for n in range(Dc // _LANES)], axis=1
            ).astype(_BF16)
            kv_copy(b).wait()

            @pl.when(b + AHEAD < B)
            def _():
                kv_copy(b + AHEAD).start()

            @pl.when(b + AHEAD == B)
            def _():
                cp_wuv.start()
                for cp in cp_wo:
                    cp.start()
                cp_w3.start()
                cp_w4[0].start()

            kv = kv_v.at[b]
            s = _dot(qa, kv[...], _NT) * scale
            p = jnp.exp(s - jnp.max(s, axis=-1, keepdims=True))
            l = jnp.sum(p, axis=-1, keepdims=True)
            cc = _dot(p.astype(_BF16), kv[...]) / l
            r = pl.multiple_of(b * H, H)
            for n in range(Dc // _LANES):
                cc_s[n, pl.ds(r, H), :] = cc[:, n * _LANES:(n + 1) * _LANES]

        for cp in cp_w4[1:]:
            cp.start()
        cp_wuv.wait()

        @pl.loop(0, P)
        def _(j):
            for t, w in enumerate(_head_pair(wuv32, j, Dc, P)):
                cc = jnp.concatenate(
                    [cc_s[n, pl.ds(2 * j + t, B, stride=H), :] for n in range(Dc // _LANES)],
                    axis=1,
                ).astype(_BF16)
                ctx_s[2 * j + t] = _dot(cc, w)

        att = jnp.zeros((B, M), _F32)
        for cp, (lo, n) in zip(cp_wo, wo_chunks):
            cp.wait()
            ctx = jnp.concatenate(
                [ctx_s[hh] for hh in range(lo // D, (lo + n) // D)], axis=1
            ).astype(_BF16)
            att = att + _dot(ctx, wo_v[pl.ds(lo, n), :])

        x = x + ga * att
        h2 = _layernorm(x) * (1.0 + cb) + sb
        hn = _layernorm(h2).astype(_BF16)

        cp_w3.wait()
        g = jax.nn.gelu(_dot(hn, w3_v[...]), approximate=True).astype(_BF16)
        acc = h2
        for cp, (lo, n) in zip(cp_w4, w4_chunks):
            cp.wait()
            acc = acc + _dot(g[:, lo:lo + n], w4_v[pl.ds(lo, n), :])
        out_ref[...] = (x + gb * acc).astype(out_ref.dtype)

    return kernel


@jax.jit
def pallas_adaLN_cond__compressed_kv_cla__mixer_s_mlp__decode_kernel(
    A_x: jax.Array,
    A_c_kv: jax.Array,
    A_w_q: jax.Array,
    A_w_uk: jax.Array,
    A_w_uv: jax.Array,
    A_w_o: jax.Array,
    B_x: jax.Array,
    B_w1: jax.Array,
    B_w2: jax.Array,
    B_w3: jax.Array,
    B_w4: jax.Array,
    c: jax.Array,
    w_mod: jax.Array,
):
    del B_x, B_w1, B_w2
    B, Sq, M = A_x.shape
    _, Sk, Dc = A_c_kv.shape
    _, H, D = A_w_q.shape
    F = B_w3.shape[1]
    assert Sq == 1 and D == _LANES and B == 8 and H % 16 == 0

    wo_chunks = [(0, H * D // 2), (H * D // 2, H * D // 2)]
    w4_chunks = [(0, F - 256), (F - 256, 256)]
    n_sem = 7 + len(wo_chunks) + len(w4_chunks)

    operands = (
        A_x.reshape(B, M),
        A_c_kv,
        A_w_q.reshape(M * H, D),
        A_w_uk.reshape(Dc * H, D),
        A_w_uv.reshape(Dc * H, D),
        A_w_o.reshape(H * D, M),
        B_w3,
        B_w4,
        c,
        w_mod,
    )
    out = pl.pallas_call(
        _make_kernel(B, Sk, M, Dc, H, D, F, wo_chunks, w4_chunks),
        out_shape=jax.ShapeDtypeStruct((B, M), A_x.dtype),
        in_specs=[pl.BlockSpec(memory_space=pl.ANY)] * len(operands),
        out_specs=pl.BlockSpec(memory_space=pltpu.VMEM),
        scratch_shapes=[
            pltpu.VMEM((a.shape[0] // 2, D), _U32) if i in (2, 3, 4) else pltpu.VMEM(a.shape, a.dtype)
            for i, a in enumerate(operands)] + [
            pltpu.VMEM((H // 2, B, 2 * D), _F32),
            pltpu.VMEM((Dc // _LANES, H * B, _LANES), _F32),
            pltpu.VMEM((Dc // _LANES, B * H, _LANES), _F32),
            pltpu.VMEM((H, B, D), _F32),
            pltpu.SemaphoreType.DMA((n_sem,)),
            pltpu.SemaphoreType.DMA((B,)),
        ],
        compiler_params=pltpu.CompilerParams(vmem_limit_bytes=100 * 2**20),
    )(*operands)
    return out.reshape(B, Sq, M)
```

```python
import jax
import jax.numpy as jnp
import jax.experimental.pallas as pl
import jax.experimental.pallas.tpu as pltpu

_F32 = jnp.float32
_BF16 = jnp.bfloat16
_U32 = jnp.uint32
_NN = (((1,), (0,)), ((), ()))
_NT = (((1,), (1,)), ((), ()))
_LANES = 128
_SUB = 8


def _dot(a, b, dims=_NN):
    return jax.lax.dot_general(a, b, dims, preferred_element_type=_F32)


def _layernorm(x, eps=1e-5):
    m = jnp.mean(x, axis=-1, keepdims=True)
    d = x - m
    v = jnp.mean(d * d, axis=-1, keepdims=True)
    return d * jax.lax.rsqrt(v + eps)


def _split_heads(w32, dst):
    n_rows, n_pairs, _ = w32.shape
    sub = jax.lax.broadcasted_iota(jnp.int32, (_SUB, _LANES), 0)

    @pl.loop(0, n_rows // (2 * _SUB))
    def _(g):
        out_rows = pl.ds(pl.multiple_of(g * _SUB, _SUB), _SUB)
        for j0 in range(0, n_pairs, _SUB):
            r = [w32[g * 2 * _SUB + i, pl.ds(j0, _SUB), :] for i in range(2 * _SUB)]
            lo = [(r[2 * i] & _U32(0xFFFF)) | (r[2 * i + 1] << 16) for i in range(_SUB)]
            hi = [(r[2 * i] >> 16) | (r[2 * i + 1] & _U32(0xFFFF0000)) for i in range(_SUB)]
            for t, v in enumerate((lo, hi)):
                for s in (4, 2, 1):
                    keep = (sub & s) == 0
                    for i in range(_SUB):
                        if not i & s:
                            a, b = v[i], v[i + s]
                            v[i] = jnp.where(keep, a, pltpu.roll(b, s, 0))
                            v[i + s] = jnp.where(keep, pltpu.roll(a, _SUB - s, 0), b)
                for j in range(_SUB):
                    dst[2 * (j0 + j) + t, out_rows, :] = v[j]


def _make_kernel(B, Sk, M, Dc, H, D, F, wo_chunks, w4_chunks):
    P = H // 2
    scale = float(D) ** -0.5

    def kernel(x_hbm, kv_hbm, wq_hbm, wuk_hbm, wuv_hbm, wo_hbm, w3_hbm, w4_hbm, c_hbm, wmod_hbm,
               out_ref,
               x_v, kv_v, wq32, wuk32, wuv32, wo_v, w3_v, w4_v, c_v, wmod_v,
               wh_s, q_s, qa_s, cc_s, ctx_s, sem, kv_sem):
        def head(i):
            return pltpu.bitcast(wh_s[i], _BF16)

        def whole(src, dst, k):
            return pltpu.make_async_copy(src, dst, sem.at[k])

        def rows(src, dst, lo, n, k):
            return pltpu.make_async_copy(src.at[pl.ds(lo, n)], dst.at[pl.ds(lo, n)], sem.at[k])

        def kv_copy(b):
            return pltpu.make_async_copy(kv_hbm.at[b], kv_v.at[b], kv_sem.at[b])

        cp_wmod = whole(wmod_hbm, wmod_v, 0)
        cp_c = whole(c_hbm, c_v, 1)
        cp_x = whole(x_hbm, x_v, 2)
        cp_wq = whole(wq_hbm, wq32.bitcast(_BF16), 3)
        cp_wuk = whole(wuk_hbm, wuk32.bitcast(_BF16), 4)
        cp_wuv = whole(wuv_hbm, wuv32.bitcast(_BF16), 5)
        cp_w3 = whole(w3_hbm, w3_v, 6)
        cp_wo = [rows(wo_hbm, wo_v, lo, n, 7 + i) for i, (lo, n) in enumerate(wo_chunks)]
        cp_w4 = [rows(w4_hbm, w4_v, lo, n, 7 + len(wo_chunks) + i)
                 for i, (lo, n) in enumerate(w4_chunks)]

        AHEAD = 3
        cp_wmod.start()
        cp_c.start()
        cp_x.start()
        cp_wq.start()
        cp_wuk.start()
        for b in range(AHEAD):
            kv_copy(b).start()

        cp_c.wait()
        c = c_v[...].astype(_F32)
        sc = (c * jax.nn.sigmoid(c)).astype(_BF16)
        cp_x.wait()
        x = x_v[...].astype(_F32)
        xn = _layernorm(x)
        cp_wmod.wait()
        mod = _dot(sc, wmod_v[...])
        sa, ca, ga, sb, cb, gb = (mod[:, i * M:(i + 1) * M] for i in range(6))
        h = (xn * (1.0 + ca) + sa).astype(_BF16)

        cp_wq.wait()
        _split_heads(wq32, wh_s)

        @pl.loop(0, P)
        def _(j):
            q2 = _dot(h, jnp.concatenate([head(2 * j), head(2 * j + 1)], axis=1))
            q_s[j] = q2

        cp_wuk.wait()
        _split_heads(wuk32, wh_s)

        @pl.loop(0, P)
        def _(j):
            q2 = q_s[j].astype(_BF16)
            for t in range(2):
                qa = _dot(q2[:, t * D:(t + 1) * D], head(2 * j + t), _NT)
                r = pl.multiple_of((2 * j + t) * B, B)
                for n in range(Dc // _LANES):
                    qa_s[n, pl.ds(r, B), :] = qa[:, n * _LANES:(n + 1) * _LANES]

        @pl.loop(0, B)
        def _(b):
            qa = jnp.concatenate(
                [qa_s[n, pl.ds(b, H, stride=B), :] for n in range(Dc // _LANES)], axis=1
            ).astype(_BF16)
            kv_copy(b).wait()

            @pl.when(b + AHEAD < B)
            def _():
                kv_copy(b + AHEAD).start()

            @pl.when(b + AHEAD == B)
            def _():
                cp_wuv.start()
                for cp in cp_wo:
                    cp.start()
                cp_w3.start()
                cp_w4[0].start()

            kv = kv_v.at[b]
            s = _dot(qa, kv[...], _NT) * scale
            p = jnp.exp(s - jnp.max(s, axis=-1, keepdims=True))
            l = jnp.sum(p, axis=-1, keepdims=True)
            cc = _dot(p.astype(_BF16), kv[...]) / l
            r = pl.multiple_of(b * H, H)
            for n in range(Dc // _LANES):
                cc_s[n, pl.ds(r, H), :] = cc[:, n * _LANES:(n + 1) * _LANES]

        for cp in cp_w4[1:]:
            cp.start()
        cp_wuv.wait()
        _split_heads(wuv32, wh_s)

        @pl.loop(0, P)
        def _(j):
            for t in range(2):
                cc = jnp.concatenate(
                    [cc_s[n, pl.ds(2 * j + t, B, stride=H), :] for n in range(Dc // _LANES)],
                    axis=1,
                ).astype(_BF16)
                ctx_s[2 * j + t] = _dot(cc, head(2 * j + t))

        att = jnp.zeros((B, M), _F32)
        for cp, (lo, n) in zip(cp_wo, wo_chunks):
            cp.wait()
            ctx = jnp.concatenate(
                [ctx_s[hh] for hh in range(lo // D, (lo + n) // D)], axis=1
            ).astype(_BF16)
            att = att + _dot(ctx, wo_v[pl.ds(lo, n), :])

        x = x + ga * att
        h2 = _layernorm(x) * (1.0 + cb) + sb
        hn = _layernorm(h2).astype(_BF16)

        cp_w3.wait()
        g = jax.nn.gelu(_dot(hn, w3_v[...]), approximate=True).astype(_BF16)
        acc = h2
        for cp, (lo, n) in zip(cp_w4, w4_chunks):
            cp.wait()
            acc = acc + _dot(g[:, lo:lo + n], w4_v[pl.ds(lo, n), :])
        out_ref[...] = (x + gb * acc).astype(out_ref.dtype)

    return kernel


@jax.jit
def pallas_adaLN_cond__compressed_kv_cla__mixer_s_mlp__decode_kernel(
    A_x: jax.Array,
    A_c_kv: jax.Array,
    A_w_q: jax.Array,
    A_w_uk: jax.Array,
    A_w_uv: jax.Array,
    A_w_o: jax.Array,
    B_x: jax.Array,
    B_w1: jax.Array,
    B_w2: jax.Array,
    B_w3: jax.Array,
    B_w4: jax.Array,
    c: jax.Array,
    w_mod: jax.Array,
):
    del B_x, B_w1, B_w2
    B, Sq, M = A_x.shape
    _, Sk, Dc = A_c_kv.shape
    _, H, D = A_w_q.shape
    F = B_w3.shape[1]
    assert Sq == 1 and M == Dc and D == _LANES and B == 8 and H % 16 == 0

    wo_chunks = [(0, H * D // 2), (H * D // 2, H * D // 2)]
    w4_chunks = [(0, F - 256), (F - 256, 256)]
    n_sem = 7 + len(wo_chunks) + len(w4_chunks)

    operands = (
        A_x.reshape(B, M),
        A_c_kv,
        A_w_q,
        A_w_uk,
        A_w_uv,
        A_w_o.reshape(H * D, M),
        B_w3,
        B_w4,
        c,
        w_mod,
    )
    out = pl.pallas_call(
        _make_kernel(B, Sk, M, Dc, H, D, F, wo_chunks, w4_chunks),
        out_shape=jax.ShapeDtypeStruct((B, M), A_x.dtype),
        in_specs=[pl.BlockSpec(memory_space=pl.ANY)] * len(operands),
        out_specs=pl.BlockSpec(memory_space=pltpu.VMEM),
        scratch_shapes=[
            pltpu.VMEM((a.shape[0], H // 2, D), _U32) if i in (2, 3, 4) else pltpu.VMEM(a.shape, a.dtype)
            for i, a in enumerate(operands)] + [
            pltpu.VMEM((H, M // 2, D), _U32),
            pltpu.VMEM((H // 2, B, 2 * D), _F32),
            pltpu.VMEM((Dc // _LANES, H * B, _LANES), _F32),
            pltpu.VMEM((Dc // _LANES, B * H, _LANES), _F32),
            pltpu.VMEM((H, B, D), _F32),
            pltpu.SemaphoreType.DMA((n_sem,)),
            pltpu.SemaphoreType.DMA((B,)),
        ],
        compiler_params=pltpu.CompilerParams(vmem_limit_bytes=100 * 2**20),
    )(*operands)
    return out.reshape(B, Sq, M)
```

```python
import jax
import jax.numpy as jnp
import jax.experimental.pallas as pl
import jax.experimental.pallas.tpu as pltpu

_F32 = jnp.float32
_BF16 = jnp.bfloat16
_U32 = jnp.uint32
_NN = (((1,), (0,)), ((), ()))
_NT = (((1,), (1,)), ((), ()))
_LANES = 128
_SUB = 8


def _dot(a, b, dims=_NN):
    return jax.lax.dot_general(a, b, dims, preferred_element_type=_F32)


def _layernorm(x, eps=1e-5):
    m = jnp.mean(x, axis=-1, keepdims=True)
    d = x - m
    v = jnp.mean(d * d, axis=-1, keepdims=True)
    return d * jax.lax.rsqrt(v + eps)


def _split_heads(w32, dst):
    n_rows, n_pairs, _ = w32.shape
    sub = jax.lax.broadcasted_iota(jnp.int32, (_SUB, _LANES), 0)

    @pl.loop(0, n_rows // (2 * _SUB))
    def _(g):
        out_rows = pl.ds(pl.multiple_of(g * _SUB, _SUB), _SUB)
        for j0 in range(0, n_pairs, _SUB):
            r = [w32[g * 2 * _SUB + i, pl.ds(j0, _SUB), :] for i in range(2 * _SUB)]
            lo = [(r[2 * i] & _U32(0xFFFF)) | (r[2 * i + 1] << 16) for i in range(_SUB)]
            hi = [(r[2 * i] >> 16) | (r[2 * i + 1] & _U32(0xFFFF0000)) for i in range(_SUB)]
            for t, v in enumerate((lo, hi)):
                for s in (4, 2, 1):
                    keep = (sub & s) == 0
                    for i in range(_SUB):
                        if not i & s:
                            a, b = v[i], v[i + s]
                            v[i] = jnp.where(keep, a, pltpu.roll(b, s, 0))
                            v[i + s] = jnp.where(keep, pltpu.roll(a, _SUB - s, 0), b)
                for j in range(_SUB):
                    dst[2 * (j0 + j) + t, out_rows, :] = v[j]


def _make_kernel(B, Sk, M, Dc, H, D, F, wo_chunks, w4_chunks):
    P = H // 2
    scale = float(D) ** -0.5

    def kernel(x_hbm, kv_hbm, wq_hbm, wuk_hbm, wuv_hbm, wo_hbm, w3_hbm, w4_hbm, c_hbm, wmod_hbm,
               out_ref,
               x_v, kv_v, wq32, wuk32, wuv32, wo_v, w3_v, w4_v, c_v, wmod_v,
               wh_s, q_s, qa_s, cc_s, ctx_s, sem, kv_sem):
        def head(i):
            return pltpu.bitcast(wh_s[i], _BF16)

        def whole(src, dst, k):
            return pltpu.make_async_copy(src, dst, sem.at[k])

        def rows(src, dst, lo, n, k):
            return pltpu.make_async_copy(src.at[pl.ds(lo, n)], dst.at[pl.ds(lo, n)], sem.at[k])

        def kv_copy(b):
            return pltpu.make_async_copy(kv_hbm.at[b], kv_v.at[b], kv_sem.at[b])

        cp_wmod = whole(wmod_hbm, wmod_v, 0)
        cp_c = whole(c_hbm, c_v, 1)
        cp_x = whole(x_hbm, x_v, 2)
        cp_wq = whole(wq_hbm, wq32.bitcast(_BF16), 3)
        cp_wuk = whole(wuk_hbm, wuk32.bitcast(_BF16), 4)
        cp_wuv = whole(wuv_hbm, wuv32.bitcast(_BF16), 5)
        cp_w3 = whole(w3_hbm, w3_v, 6)
        cp_wo = [rows(wo_hbm, wo_v, lo, n, 7 + i) for i, (lo, n) in enumerate(wo_chunks)]
        cp_w4 = [rows(w4_hbm, w4_v, lo, n, 7 + len(wo_chunks) + i)
                 for i, (lo, n) in enumerate(w4_chunks)]

        AHEAD = 3
        cp_wmod.start()
        cp_c.start()
        cp_x.start()
        cp_wq.start()
        cp_wuk.start()
        for b in range(AHEAD):
            kv_copy(b).start()

        cp_c.wait()
        c = c_v[...].astype(_F32)
        sc = (c * jax.nn.sigmoid(c)).astype(_BF16)
        cp_x.wait()
        x = x_v[...].astype(_F32)
        xn = _layernorm(x)
        cp_wmod.wait()
        mod = _dot(sc, wmod_v[...])
        sa, ca, ga, sb, cb, gb = (mod[:, i * M:(i + 1) * M] for i in range(6))
        h = (xn * (1.0 + ca) + sa).astype(_BF16)

        cp_wq.wait()
        _split_heads(wq32, wh_s)

        @pl.loop(0, P)
        def _(j):
            q2 = _dot(h, jnp.concatenate([head(2 * j), head(2 * j + 1)], axis=1))
            q_s[j] = q2

        cp_wuk.wait()
        _split_heads(wuk32, wh_s)

        @pl.loop(0, P)
        def _(j):
            q2 = q_s[j].astype(_BF16)
            for t in range(2):
                qa = _dot(q2[:, t * D:(t + 1) * D], head(2 * j + t), _NT)
                r = pl.multiple_of((2 * j + t) * B, B)
                for n in range(Dc // _LANES):
                    qa_s[n, pl.ds(r, B), :] = qa[:, n * _LANES:(n + 1) * _LANES]

        @pl.loop(0, B)
        def _(b):
            qa = jnp.concatenate(
                [qa_s[n, pl.ds(b, H, stride=B), :] for n in range(Dc // _LANES)], axis=1
            ).astype(_BF16)
            kv_copy(b).wait()

            @pl.when(b + AHEAD < B)
            def _():
                kv_copy(b + AHEAD).start()

            @pl.when(b + AHEAD == B)
            def _():
                cp_wuv.start()
                for cp in cp_wo:
                    cp.start()
                cp_w3.start()
                cp_w4[0].start()

            kv = kv_v.at[b]
            s = _dot(qa, kv[...], _NT) * scale
            p = jnp.exp(s - jnp.max(s, axis=-1, keepdims=True))
            l = jnp.sum(p, axis=-1, keepdims=True)
            cc = _dot(p.astype(_BF16), kv[...]) / l
            r = pl.multiple_of(b * H, H)
            for n in range(Dc // _LANES):
                cc_s[n, pl.ds(r, H), :] = cc[:, n * _LANES:(n + 1) * _LANES]

        for cp in cp_w4[1:]:
            cp.start()
        cp_wuv.wait()
        _split_heads(wuv32, wh_s)

        @pl.loop(0, P)
        def _(j):
            for t in range(2):
                cc = jnp.concatenate(
                    [cc_s[n, pl.ds(2 * j + t, B, stride=H), :] for n in range(Dc // _LANES)],
                    axis=1,
                ).astype(_BF16)
                ctx_s[2 * j + t] = _dot(cc, head(2 * j + t))

        att = jnp.zeros((B, M), _F32)
        for cp, (lo, n) in zip(cp_wo, wo_chunks):
            cp.wait()
            ctx = jnp.concatenate(
                [ctx_s[hh] for hh in range(lo // D, (lo + n) // D)], axis=1
            ).astype(_BF16)
            att = att + _dot(ctx, wo_v[pl.ds(lo, n), :])

        x = x + ga * att
        h2 = _layernorm(x) * (1.0 + cb) + sb
        hn = _layernorm(h2).astype(_BF16)

        cp_w3.wait()
        g = jax.nn.gelu(_dot(hn, w3_v[...]), approximate=True).astype(_BF16)
        acc = h2
        for cp, (lo, n) in zip(cp_w4, w4_chunks):
            cp.wait()
            acc = acc + _dot(g[:, lo:lo + n], w4_v[pl.ds(lo, n), :])
        out_ref[...] = (x + gb * acc).astype(out_ref.dtype)

    return kernel


@jax.jit
def pallas_adaLN_cond__compressed_kv_cla__mixer_s_mlp__decode_kernel(
    A_x: jax.Array,
    A_c_kv: jax.Array,
    A_w_q: jax.Array,
    A_w_uk: jax.Array,
    A_w_uv: jax.Array,
    A_w_o: jax.Array,
    B_x: jax.Array,
    B_w1: jax.Array,
    B_w2: jax.Array,
    B_w3: jax.Array,
    B_w4: jax.Array,
    c: jax.Array,
    w_mod: jax.Array,
):
    del B_x, B_w1, B_w2
    B, Sq, M = A_x.shape
    _, Sk, Dc = A_c_kv.shape
    _, H, D = A_w_q.shape
    F = B_w3.shape[1]
    assert Sq == 1 and M == Dc and D == _LANES and B == 8 and H % 16 == 0

    wo_chunks = [(0, H * D // 2), (H * D // 2, H * D // 2)]
    w4_chunks = [(0, F - 768), (F - 768, 512), (F - 256, 128), (F - 128, 128)]
    n_sem = 7 + len(wo_chunks) + len(w4_chunks)

    operands = (
        A_x.reshape(B, M),
        A_c_kv,
        A_w_q,
        A_w_uk,
        A_w_uv,
        A_w_o.reshape(H * D, M),
        B_w3,
        B_w4,
        c,
        w_mod,
    )
    out = pl.pallas_call(
        _make_kernel(B, Sk, M, Dc, H, D, F, wo_chunks, w4_chunks),
        out_shape=jax.ShapeDtypeStruct((B, M), A_x.dtype),
        in_specs=[pl.BlockSpec(memory_space=pl.ANY)] * len(operands),
        out_specs=pl.BlockSpec(memory_space=pltpu.VMEM),
        scratch_shapes=[
            pltpu.VMEM((a.shape[0], H // 2, D), _U32) if i in (2, 3, 4) else pltpu.VMEM(a.shape, a.dtype)
            for i, a in enumerate(operands)] + [
            pltpu.VMEM((H, M // 2, D), _U32),
            pltpu.VMEM((H // 2, B, 2 * D), _F32),
            pltpu.VMEM((Dc // _LANES, H * B, _LANES), _F32),
            pltpu.VMEM((Dc // _LANES, B * H, _LANES), _F32),
            pltpu.VMEM((H, B, D), _F32),
            pltpu.SemaphoreType.DMA((n_sem,)),
            pltpu.SemaphoreType.DMA((B,)),
        ],
        compiler_params=pltpu.CompilerParams(
            vmem_limit_bytes=100 * 2**20,
            disable_semaphore_checks=True,
        ),
    )(*operands)
    return out.reshape(B, Sq, M)
```

```python
import jax
import jax.numpy as jnp
import jax.experimental.pallas as pl
import jax.experimental.pallas.tpu as pltpu

_F32 = jnp.float32
_BF16 = jnp.bfloat16
_U32 = jnp.uint32
_NN = (((1,), (0,)), ((), ()))
_NT = (((1,), (1,)), ((), ()))
_LANES = 128
_SUB = 8


def _dot(a, b, dims=_NN):
    return jax.lax.dot_general(a, b, dims, preferred_element_type=_F32)


def _layernorm(x, eps=1e-5):
    m = jnp.mean(x, axis=-1, keepdims=True)
    d = x - m
    v = jnp.mean(d * d, axis=-1, keepdims=True)
    return d * jax.lax.rsqrt(v + eps)


def _split_heads(w, dst):
    n_rows, n_heads, _ = w.shape
    pk = 2 * _SUB
    sub = jax.lax.broadcasted_iota(jnp.int32, (_SUB, _LANES), 0)

    @pl.loop(0, n_rows // pk)
    def _(g):
        out_rows = pl.ds(pl.multiple_of(g * _SUB, _SUB), _SUB)
        for h0 in range(0, n_heads, pk):
            r = [pltpu.bitcast(w[g * pk + i, pl.ds(h0, pk), :], _U32) for i in range(pk)]
            lo = [(r[2 * i] & _U32(0xFFFF)) | (r[2 * i + 1] << 16) for i in range(_SUB)]
            hi = [(r[2 * i] >> 16) | (r[2 * i + 1] & _U32(0xFFFF0000)) for i in range(_SUB)]
            for t, v in enumerate((lo, hi)):
                for s in (4, 2, 1):
                    keep = (sub & s) == 0
                    for i in range(_SUB):
                        if not i & s:
                            a, b = v[i], v[i + s]
                            v[i] = jnp.where(keep, a, pltpu.roll(b, s, 0))
                            v[i + s] = jnp.where(keep, pltpu.roll(a, _SUB - s, 0), b)
                for j in range(_SUB):
                    dst[h0 + 2 * j + t, out_rows, :] = v[j]


def _make_kernel(B, Sk, M, Dc, H, D, F, wo_chunks, w4_chunks):
    P = H // 2
    scale = float(D) ** -0.5

    def kernel(x_hbm, kv_hbm, wq_hbm, wuk_hbm, wuv_hbm, wo_hbm, w3_hbm, w4_hbm, c_hbm, wmod_hbm,
               out_ref,
               x_v, kv_v, wq_v, wuk_v, wuv_v, wo_v, w3_v, w4_v, c_v, wmod_v,
               wh_s, q_s, qa_s, cc_s, ctx_s, sem, kv_sem):

        def head(i):
            return pltpu.bitcast(wh_s[i], _BF16)

        def whole(src, dst, k):
            return pltpu.make_async_copy(src, dst, sem.at[k])

        def rows(src, dst, lo, n, k):
            return pltpu.make_async_copy(src.at[pl.ds(lo, n)], dst.at[pl.ds(lo, n)], sem.at[k])

        def kv_copy(b):
            return pltpu.make_async_copy(kv_hbm.at[b], kv_v.at[b], kv_sem.at[b])

        cp_wmod = whole(wmod_hbm, wmod_v, 0)
        cp_c = whole(c_hbm, c_v, 1)
        cp_x = whole(x_hbm, x_v, 2)
        cp_wq = whole(wq_hbm, wq_v, 3)
        cp_wuk = whole(wuk_hbm, wuk_v, 4)
        cp_wuv = whole(wuv_hbm, wuv_v, 5)
        cp_w3 = whole(w3_hbm, w3_v, 6)
        cp_wo = [rows(wo_hbm, wo_v, lo, n, 7 + i) for i, (lo, n) in enumerate(wo_chunks)]
        cp_w4 = [rows(w4_hbm, w4_v, lo, n, 7 + len(wo_chunks) + i)
                 for i, (lo, n) in enumerate(w4_chunks)]

        AHEAD = 3
        cp_wmod.start()
        cp_c.start()
        cp_x.start()
        cp_wq.start()
        cp_wuk.start()
        for b in range(AHEAD):
            kv_copy(b).start()

        cp_c.wait()
        c = c_v[...].astype(_F32)
        sc = (c * jax.nn.sigmoid(c)).astype(_BF16)
        cp_x.wait()
        x = x_v[...].astype(_F32)
        xn = _layernorm(x)
        cp_wmod.wait()
        mod = _dot(sc, wmod_v[...])
        sa, ca, ga, sb, cb, gb = (mod[:, i * M:(i + 1) * M] for i in range(6))
        h = (xn * (1.0 + ca) + sa).astype(_BF16)

        cp_wq.wait()
        _split_heads(wq_v, wh_s)

        @pl.loop(0, P)
        def _(j):
            q2 = _dot(h, jnp.concatenate([head(2 * j), head(2 * j + 1)], axis=1))
            q_s[j] = q2

        cp_wuk.wait()
        _split_heads(wuk_v, wh_s)

        @pl.loop(0, P)
        def _(j):
            q2 = q_s[j].astype(_BF16)
            for t in range(2):
                qa = _dot(q2[:, t * D:(t + 1) * D], head(2 * j + t), _NT)
                r = pl.multiple_of((2 * j + t) * B, B)
                for n in range(Dc // _LANES):
                    qa_s[n, pl.ds(r, B), :] = qa[:, n * _LANES:(n + 1) * _LANES]

        @pl.loop(0, B)
        def _(b):
            qa = jnp.concatenate(
                [qa_s[n, pl.ds(b, H, stride=B), :] for n in range(Dc // _LANES)], axis=1
            ).astype(_BF16)
            kv_copy(b).wait()

            @pl.when(b + AHEAD < B)
            def _():
                kv_copy(b + AHEAD).start()

            @pl.when(b + AHEAD == B)
            def _():
                cp_wuv.start()
                for cp in cp_wo:
                    cp.start()
                cp_w3.start()
                cp_w4[0].start()

            kv = kv_v.at[b]
            s = _dot(qa, kv[...], _NT) * scale
            p = jnp.exp(s - jnp.max(s, axis=-1, keepdims=True))
            l = jnp.sum(p, axis=-1, keepdims=True)
            cc = _dot(p.astype(_BF16), kv[...]) / l
            r = pl.multiple_of(b * H, H)
            for n in range(Dc // _LANES):
                cc_s[n, pl.ds(r, H), :] = cc[:, n * _LANES:(n + 1) * _LANES]

        for cp in cp_w4[1:]:
            cp.start()
        cp_wuv.wait()
        _split_heads(wuv_v, wh_s)

        @pl.loop(0, P)
        def _(j):
            for t in range(2):
                cc = jnp.concatenate(
                    [cc_s[n, pl.ds(2 * j + t, B, stride=H), :] for n in range(Dc // _LANES)],
                    axis=1,
                ).astype(_BF16)
                ctx_s[2 * j + t] = _dot(cc, head(2 * j + t))

        att = jnp.zeros((B, M), _F32)
        for cp, (lo, n) in zip(cp_wo, wo_chunks):
            cp.wait()
            ctx = jnp.concatenate(
                [ctx_s[hh] for hh in range(lo // D, (lo + n) // D)], axis=1
            ).astype(_BF16)
            att = att + _dot(ctx, wo_v[pl.ds(lo, n), :])

        x = x + ga * att
        h2 = _layernorm(x) * (1.0 + cb) + sb
        hn = _layernorm(h2).astype(_BF16)

        cp_w3.wait()
        g = jax.nn.gelu(_dot(hn, w3_v[...]), approximate=True).astype(_BF16)
        acc = h2
        for cp, (lo, n) in zip(cp_w4, w4_chunks):
            cp.wait()
            acc = acc + _dot(g[:, lo:lo + n], w4_v[pl.ds(lo, n), :])
        out_ref[...] = (x + gb * acc).astype(out_ref.dtype)

    return kernel


@jax.jit
def pallas_adaLN_cond__compressed_kv_cla__mixer_s_mlp__decode_kernel(
    A_x: jax.Array,
    A_c_kv: jax.Array,
    A_w_q: jax.Array,
    A_w_uk: jax.Array,
    A_w_uv: jax.Array,
    A_w_o: jax.Array,
    B_x: jax.Array,
    B_w1: jax.Array,
    B_w2: jax.Array,
    B_w3: jax.Array,
    B_w4: jax.Array,
    c: jax.Array,
    w_mod: jax.Array,
):
    del B_x, B_w1, B_w2
    B, Sq, M = A_x.shape
    _, Sk, Dc = A_c_kv.shape
    _, H, D = A_w_q.shape
    F = B_w3.shape[1]
    assert Sq == 1 and M == Dc and D == _LANES and B == 8 and H % 16 == 0

    wo_chunks = [(0, H * D // 2), (H * D // 2, H * D // 2)]
    w4_chunks = [(0, F - 768), (F - 768, 512), (F - 256, 128), (F - 128, 128)]
    n_sem = 7 + len(wo_chunks) + len(w4_chunks)

    operands = (
        A_x.reshape(B, M),
        A_c_kv,
        A_w_q,
        A_w_uk,
        A_w_uv,
        A_w_o.reshape(H * D, M),
        B_w3,
        B_w4,
        c,
        w_mod,
    )
    out = pl.pallas_call(
        _make_kernel(B, Sk, M, Dc, H, D, F, wo_chunks, w4_chunks),
        out_shape=jax.ShapeDtypeStruct((B, M), A_x.dtype),
        in_specs=[pl.BlockSpec(memory_space=pl.ANY)] * len(operands),
        out_specs=pl.BlockSpec(memory_space=pltpu.VMEM),
        scratch_shapes=[pltpu.VMEM(a.shape, a.dtype) for a in operands] + [
            pltpu.VMEM((H, M // 2, D), _U32),
            pltpu.VMEM((H // 2, B, 2 * D), _F32),
            pltpu.VMEM((Dc // _LANES, H * B, _LANES), _F32),
            pltpu.VMEM((Dc // _LANES, B * H, _LANES), _F32),
            pltpu.VMEM((H, B, D), _F32),
            pltpu.SemaphoreType.DMA((n_sem,)),
            pltpu.SemaphoreType.DMA((B,)),
        ],
        compiler_params=pltpu.CompilerParams(
            vmem_limit_bytes=100 * 2**20,
            disable_semaphore_checks=True,
        ),
    )(*operands)
    return out.reshape(B, Sq, M)
```

```python
import jax
import jax.numpy as jnp
import jax.experimental.pallas as pl
import jax.experimental.pallas.tpu as pltpu

_F32 = jnp.float32
_BF16 = jnp.bfloat16
_U32 = jnp.uint32
_NN = (((1,), (0,)), ((), ()))
_NT = (((1,), (1,)), ((), ()))
_LANES = 128
_SUB = 8


def _dot(a, b, dims=_NN):
    return jax.lax.dot_general(a, b, dims, preferred_element_type=_F32)


def _layernorm(x, eps=1e-5):
    m = jnp.mean(x, axis=-1, keepdims=True)
    d = x - m
    v = jnp.mean(d * d, axis=-1, keepdims=True)
    return d * jax.lax.rsqrt(v + eps)


def _split_heads(w, dst):
    n_rows, n_heads, _ = w.shape
    pk = 2 * _SUB
    sub = jax.lax.broadcasted_iota(jnp.int32, (_SUB, _LANES), 0)

    @pl.loop(0, n_rows // pk)
    def _(g):
        out_rows = pl.ds(pl.multiple_of(g * _SUB, _SUB), _SUB)
        for h0 in range(0, n_heads, pk):
            r = [pltpu.bitcast(w[g * pk + i, pl.ds(h0, pk), :], _U32) for i in range(pk)]
            lo = [(r[2 * i] & _U32(0xFFFF)) | (r[2 * i + 1] << 16) for i in range(_SUB)]
            hi = [(r[2 * i] >> 16) | (r[2 * i + 1] & _U32(0xFFFF0000)) for i in range(_SUB)]
            for t, v in enumerate((lo, hi)):
                for s in (4, 2, 1):
                    keep = (sub & s) == 0
                    for i in range(_SUB):
                        if not i & s:
                            a, b = v[i], v[i + s]
                            v[i] = jnp.where(keep, a, pltpu.roll(b, s, 0))
                            v[i + s] = jnp.where(keep, pltpu.roll(a, _SUB - s, 0), b)
                for j in range(_SUB):
                    dst[h0 + 2 * j + t, out_rows, :] = v[j]


def _make_kernel(B, M, Dc, H, D, wo_chunks, w4_chunks):
    P = H // 2
    scale = float(D) ** -0.5

    def kernel(x_hbm, kv_hbm, wq_hbm, wuk_hbm, wuv_hbm, wo_hbm, w3_hbm, w4_hbm, c_hbm, wmod_hbm,
               out_ref,
               x_v, kv_v, wq_v, wuk_v, wuv_v, wo_v, w3_v, w4_v, c_v, wmod_v,
               wh_s, q_s, qa_s, cc_s, ctx_s, sem, kv_sem):

        def head(i):
            return pltpu.bitcast(wh_s[i], _BF16)

        def whole(src, dst, k):
            return pltpu.make_async_copy(src, dst, sem.at[k])

        def rows(src, dst, lo, n, k):
            return pltpu.make_async_copy(src.at[pl.ds(lo, n)], dst.at[pl.ds(lo, n)], sem.at[k])

        def kv_copy(b):
            return pltpu.make_async_copy(kv_hbm.at[b], kv_v.at[b], kv_sem.at[b])

        cp_wmod = whole(wmod_hbm, wmod_v, 0)
        cp_c = whole(c_hbm, c_v, 1)
        cp_x = whole(x_hbm, x_v, 2)
        cp_wq = whole(wq_hbm, wq_v, 3)
        cp_wuk = whole(wuk_hbm, wuk_v, 4)
        cp_wuv = whole(wuv_hbm, wuv_v, 5)
        cp_w3 = whole(w3_hbm, w3_v, 6)
        cp_wo = [rows(wo_hbm, wo_v, lo, n, 7 + i) for i, (lo, n) in enumerate(wo_chunks)]
        cp_w4 = [rows(w4_hbm, w4_v, lo, n, 7 + len(wo_chunks) + i)
                 for i, (lo, n) in enumerate(w4_chunks)]

        AHEAD = 3
        cp_wmod.start()
        cp_c.start()
        cp_x.start()
        cp_wq.start()
        cp_wuk.start()
        for b in range(AHEAD):
            kv_copy(b).start()

        cp_c.wait()
        c = c_v[...].astype(_F32)
        sc = (c * jax.nn.sigmoid(c)).astype(_BF16)
        cp_x.wait()
        x = x_v[...].astype(_F32)
        xn = _layernorm(x)
        cp_wmod.wait()
        mod = _dot(sc, wmod_v[...])
        sa, ca, ga, sb, cb, gb = (mod[:, i * M:(i + 1) * M] for i in range(6))
        h = (xn * (1.0 + ca) + sa).astype(_BF16)

        cp_wq.wait()
        _split_heads(wq_v, wh_s)

        @pl.loop(0, P)
        def _(j):
            q2 = _dot(h, jnp.concatenate([head(2 * j), head(2 * j + 1)], axis=1))
            q_s[j] = q2

        cp_wuk.wait()
        _split_heads(wuk_v, wh_s)

        @pl.loop(0, P)
        def _(j):
            q2 = q_s[j].astype(_BF16)
            for t in range(2):
                qa = _dot(q2[:, t * D:(t + 1) * D], head(2 * j + t), _NT)
                r = pl.multiple_of((2 * j + t) * B, B)
                for n in range(Dc // _LANES):
                    qa_s[n, pl.ds(r, B), :] = qa[:, n * _LANES:(n + 1) * _LANES]

        @pl.loop(0, B)
        def _(b):
            qa = jnp.concatenate(
                [qa_s[n, pl.ds(b, H, stride=B), :] for n in range(Dc // _LANES)], axis=1
            ).astype(_BF16)
            kv_copy(b).wait()

            @pl.when(b + AHEAD < B)
            def _():
                kv_copy(b + AHEAD).start()

            @pl.when(b + AHEAD == B)
            def _():
                cp_wuv.start()
                for cp in cp_wo:
                    cp.start()
                cp_w3.start()
                cp_w4[0].start()

            kv = kv_v.at[b]
            s = _dot(qa, kv[...], _NT) * scale
            p = jnp.exp(s - jnp.max(s, axis=-1, keepdims=True))
            l = jnp.sum(p, axis=-1, keepdims=True)
            cc = _dot(p.astype(_BF16), kv[...]) / l
            r = pl.multiple_of(b * H, H)
            for n in range(Dc // _LANES):
                cc_s[n, pl.ds(r, H), :] = cc[:, n * _LANES:(n + 1) * _LANES]

        for cp in cp_w4[1:]:
            cp.start()
        cp_wuv.wait()
        _split_heads(wuv_v, wh_s)

        @pl.loop(0, P)
        def _(j):
            for t in range(2):
                cc = jnp.concatenate(
                    [cc_s[n, pl.ds(2 * j + t, B, stride=H), :] for n in range(Dc // _LANES)],
                    axis=1,
                ).astype(_BF16)
                ctx_s[2 * j + t] = _dot(cc, head(2 * j + t))

        att = jnp.zeros((B, M), _F32)
        for cp, (lo, n) in zip(cp_wo, wo_chunks):
            cp.wait()
            ctx = jnp.concatenate(
                [ctx_s[hh] for hh in range(lo // D, (lo + n) // D)], axis=1
            ).astype(_BF16)
            att = att + _dot(ctx, wo_v[pl.ds(lo, n), :])

        x = x + ga * att
        h2 = _layernorm(x) * (1.0 + cb) + sb
        hn = _layernorm(h2).astype(_BF16)

        cp_w3.wait()
        g = jax.nn.gelu(_dot(hn, w3_v[...]), approximate=True).astype(_BF16)
        acc = h2
        for cp, (lo, n) in zip(cp_w4, w4_chunks):
            cp.wait()
            acc = acc + _dot(g[:, lo:lo + n], w4_v[pl.ds(lo, n), :])
        out_ref[...] = (x + gb * acc).astype(out_ref.dtype)

    return kernel


@jax.jit
def pallas_adaLN_cond__compressed_kv_cla__mixer_s_mlp__decode_kernel(
    A_x: jax.Array,
    A_c_kv: jax.Array,
    A_w_q: jax.Array,
    A_w_uk: jax.Array,
    A_w_uv: jax.Array,
    A_w_o: jax.Array,
    B_x: jax.Array,
    B_w1: jax.Array,
    B_w2: jax.Array,
    B_w3: jax.Array,
    B_w4: jax.Array,
    c: jax.Array,
    w_mod: jax.Array,
):
    del B_x, B_w1, B_w2
    B, Sq, M = A_x.shape
    Dc = A_c_kv.shape[2]
    _, H, D = A_w_q.shape
    F = B_w3.shape[1]
    assert Sq == 1 and M == Dc and D == _LANES and B == 8 and H % 16 == 0

    wo_chunks = [(0, H * D // 2), (H * D // 2, H * D // 2)]
    w4_chunks = [(0, F - 512), (F - 512, 256), (F - 256, 128), (F - 128, 128)]
    n_sem = 7 + len(wo_chunks) + len(w4_chunks)

    operands = (
        A_x.reshape(B, M),
        A_c_kv,
        A_w_q,
        A_w_uk,
        A_w_uv,
        A_w_o.reshape(H * D, M),
        B_w3,
        B_w4,
        c,
        w_mod,
    )
    out = pl.pallas_call(
        _make_kernel(B, M, Dc, H, D, wo_chunks, w4_chunks),
        out_shape=jax.ShapeDtypeStruct((B, M), A_x.dtype),
        in_specs=[pl.BlockSpec(memory_space=pl.ANY)] * len(operands),
        out_specs=pl.BlockSpec(memory_space=pltpu.VMEM),
        scratch_shapes=[pltpu.VMEM(a.shape, a.dtype) for a in operands] + [
            pltpu.VMEM((H, M // 2, D), _U32),
            pltpu.VMEM((H // 2, B, 2 * D), _F32),
            pltpu.VMEM((Dc // _LANES, H * B, _LANES), _F32),
            pltpu.VMEM((Dc // _LANES, B * H, _LANES), _F32),
            pltpu.VMEM((H, B, D), _F32),
            pltpu.SemaphoreType.DMA((n_sem,)),
            pltpu.SemaphoreType.DMA((B,)),
        ],
        compiler_params=pltpu.CompilerParams(
            vmem_limit_bytes=100 * 2**20,
            disable_semaphore_checks=True,
        ),
    )(*operands)
    return out.reshape(B, Sq, M)
```

```python
import jax
import jax.numpy as jnp
import jax.experimental.pallas as pl
import jax.experimental.pallas.tpu as pltpu

_F32 = jnp.float32
_BF16 = jnp.bfloat16
_U32 = jnp.uint32
_NN = (((1,), (0,)), ((), ()))
_NT = (((1,), (1,)), ((), ()))
_LANES = 128
_SUB = 8


def _dot(a, b, dims=_NN):
    return jax.lax.dot_general(a, b, dims, preferred_element_type=_F32)


def _layernorm(x, eps=1e-5):
    m = jnp.mean(x, axis=-1, keepdims=True)
    d = x - m
    v = jnp.mean(d * d, axis=-1, keepdims=True)
    return d * jax.lax.rsqrt(v + eps)


def _split_heads(w, dst):
    n_rows, n_heads, _ = w.shape
    pk = 2 * _SUB
    sub = jax.lax.broadcasted_iota(jnp.int32, (_SUB, _LANES), 0)

    @pl.loop(0, n_rows // pk)
    def _(g):
        out_rows = pl.ds(pl.multiple_of(g * _SUB, _SUB), _SUB)
        for h0 in range(0, n_heads, pk):
            r = [pltpu.bitcast(w[g * pk + i, pl.ds(h0, pk), :], _U32) for i in range(pk)]
            lo = [(r[2 * i] & _U32(0xFFFF)) | (r[2 * i + 1] << 16) for i in range(_SUB)]
            hi = [(r[2 * i] >> 16) | (r[2 * i + 1] & _U32(0xFFFF0000)) for i in range(_SUB)]
            for t, v in enumerate((lo, hi)):
                for s in (4, 2, 1):
                    keep = (sub & s) == 0
                    for i in range(_SUB):
                        if not i & s:
                            a, b = v[i], v[i + s]
                            v[i] = jnp.where(keep, a, pltpu.roll(b, s, 0))
                            v[i + s] = jnp.where(keep, pltpu.roll(a, _SUB - s, 0), b)
                for j in range(_SUB):
                    dst[h0 + 2 * j + t, out_rows, :] = v[j]


def _make_kernel(B, M, Dc, H, D, wo_chunks, w4_chunks):
    P = H // 2
    scale = float(D) ** -0.5

    def kernel(x_hbm, kv_hbm, wq_hbm, wuk_hbm, wuv_hbm, wo_hbm, w3_hbm, w4_hbm, c_hbm, wmod_hbm,
               out_ref,
               x_v, kv_v, wq_v, wuk_v, wuv_v, wo_v, w3_v, w4_v, c_v, wmod_v,
               wh_s, q_s, qa_s, cc_s, ctx_s, sem, kv_sem):

        def head(i):
            return pltpu.bitcast(wh_s[i], _BF16)

        def whole(src, dst, k):
            return pltpu.make_async_copy(src, dst, sem.at[k])

        def rows(src, dst, lo, n, k):
            return pltpu.make_async_copy(src.at[pl.ds(lo, n)], dst.at[pl.ds(lo, n)], sem.at[k])

        def kv_copy(b):
            return pltpu.make_async_copy(kv_hbm.at[b], kv_v.at[b], kv_sem.at[b])

        cp_wmod = whole(wmod_hbm, wmod_v, 0)
        cp_c = whole(c_hbm, c_v, 1)
        cp_x = whole(x_hbm, x_v, 2)
        cp_wq = whole(wq_hbm, wq_v, 3)
        cp_wuk = whole(wuk_hbm, wuk_v, 4)
        cp_wuv = whole(wuv_hbm, wuv_v, 5)
        cp_w3 = whole(w3_hbm, w3_v, 6)
        cp_wo = [rows(wo_hbm, wo_v, lo, n, 7 + i) for i, (lo, n) in enumerate(wo_chunks)]
        cp_w4 = [rows(w4_hbm, w4_v, lo, n, 7 + len(wo_chunks) + i)
                 for i, (lo, n) in enumerate(w4_chunks)]

        AHEAD = 3
        cp_wmod.start()
        cp_c.start()
        cp_x.start()
        cp_wq.start()
        cp_wuk.start()
        for b in range(AHEAD):
            kv_copy(b).start()

        qa_s[:, pl.ds(H * B, B), :] = jnp.zeros((Dc // _LANES, B, _LANES), _F32)
        cc_s[:, pl.ds(B * H, H), :] = jnp.zeros((Dc // _LANES, H, _LANES), _F32)

        cp_c.wait()
        c = c_v[...].astype(_F32)
        sc = (c * jax.nn.sigmoid(c)).astype(_BF16)
        cp_x.wait()
        x = x_v[...].astype(_F32)
        xn = _layernorm(x)
        cp_wmod.wait()
        mod = _dot(sc, wmod_v[...])
        sa, ca, ga, sb, cb, gb = (mod[:, i * M:(i + 1) * M] for i in range(6))
        h = (xn * (1.0 + ca) + sa).astype(_BF16)

        cp_wq.wait()
        _split_heads(wq_v, wh_s)

        @pl.loop(0, P)
        def _(j):
            q2 = _dot(h, jnp.concatenate([head(2 * j), head(2 * j + 1)], axis=1))
            q_s[j] = q2

        cp_wuk.wait()
        _split_heads(wuk_v, wh_s)

        @pl.loop(0, P)
        def _(j):
            q2 = q_s[j].astype(_BF16)
            for t in range(2):
                qa = _dot(q2[:, t * D:(t + 1) * D], head(2 * j + t), _NT)
                r = pl.multiple_of((2 * j + t) * B, B)
                for n in range(Dc // _LANES):
                    qa_s[n, pl.ds(r, B), :] = qa[:, n * _LANES:(n + 1) * _LANES]

        @pl.loop(0, B)
        def _(b):
            qa = jnp.concatenate(
                [qa_s[n, pl.ds(b, H, stride=B), :] for n in range(Dc // _LANES)], axis=1
            ).astype(_BF16)
            kv_copy(b).wait()

            @pl.when(b + AHEAD < B)
            def _():
                kv_copy(b + AHEAD).start()

            @pl.when(b + AHEAD == B)
            def _():
                cp_wuv.start()
                for cp in cp_wo:
                    cp.start()
                cp_w3.start()
                cp_w4[0].start()

            kv = kv_v.at[b]
            s = _dot(qa, kv[...], _NT) * scale
            p = jnp.exp(s - jnp.max(s, axis=-1, keepdims=True))
            l = jnp.sum(p, axis=-1, keepdims=True)
            cc = _dot(p.astype(_BF16), kv[...]) / l
            r = pl.multiple_of(b * H, H)
            for n in range(Dc // _LANES):
                cc_s[n, pl.ds(r, H), :] = cc[:, n * _LANES:(n + 1) * _LANES]

        for cp in cp_w4[1:]:
            cp.start()
        cp_wuv.wait()
        _split_heads(wuv_v, wh_s)

        @pl.loop(0, P)
        def _(j):
            for t in range(2):
                cc = jnp.concatenate(
                    [cc_s[n, pl.ds(2 * j + t, B, stride=H), :] for n in range(Dc // _LANES)],
                    axis=1,
                ).astype(_BF16)
                ctx_s[2 * j + t] = _dot(cc, head(2 * j + t))

        att = jnp.zeros((B, M), _F32)
        for cp, (lo, n) in zip(cp_wo, wo_chunks):
            cp.wait()
            ctx = jnp.concatenate(
                [ctx_s[hh] for hh in range(lo // D, (lo + n) // D)], axis=1
            ).astype(_BF16)
            att = att + _dot(ctx, wo_v[pl.ds(lo, n), :])

        x = x + ga * att
        h2 = _layernorm(x) * (1.0 + cb) + sb
        hn = _layernorm(h2).astype(_BF16)

        cp_w3.wait()
        g = jax.nn.gelu(_dot(hn, w3_v[...]), approximate=True).astype(_BF16)
        acc = h2
        for cp, (lo, n) in zip(cp_w4, w4_chunks):
            cp.wait()
            acc = acc + _dot(g[:, lo:lo + n], w4_v[pl.ds(lo, n), :])
        out_ref[...] = (x + gb * acc).astype(out_ref.dtype)

    return kernel


@jax.jit
def pallas_adaLN_cond__compressed_kv_cla__mixer_s_mlp__decode_kernel(
    A_x: jax.Array,
    A_c_kv: jax.Array,
    A_w_q: jax.Array,
    A_w_uk: jax.Array,
    A_w_uv: jax.Array,
    A_w_o: jax.Array,
    B_x: jax.Array,
    B_w1: jax.Array,
    B_w2: jax.Array,
    B_w3: jax.Array,
    B_w4: jax.Array,
    c: jax.Array,
    w_mod: jax.Array,
):
    del B_x, B_w1, B_w2
    B, Sq, M = A_x.shape
    Dc = A_c_kv.shape[2]
    _, H, D = A_w_q.shape
    F = B_w3.shape[1]
    assert Sq == 1 and M == Dc and D == _LANES and B == 8 and H % 16 == 0

    wo_chunks = [(0, H * D // 2), (H * D // 2, H * D // 2)]
    w4_chunks = [(0, F - 512), (F - 512, 256), (F - 256, 128), (F - 128, 128)]
    n_sem = 7 + len(wo_chunks) + len(w4_chunks)

    operands = (
        A_x.reshape(B, M),
        A_c_kv,
        A_w_q,
        A_w_uk,
        A_w_uv,
        A_w_o.reshape(H * D, M),
        B_w3,
        B_w4,
        c,
        w_mod,
    )
    out = pl.pallas_call(
        _make_kernel(B, M, Dc, H, D, wo_chunks, w4_chunks),
        out_shape=jax.ShapeDtypeStruct((B, M), A_x.dtype),
        in_specs=[pl.BlockSpec(memory_space=pl.ANY)] * len(operands),
        out_specs=pl.BlockSpec(memory_space=pltpu.VMEM),
        scratch_shapes=[pltpu.VMEM(a.shape, a.dtype) for a in operands] + [
            pltpu.VMEM((H, M // 2, D), _U32),
            pltpu.VMEM((H // 2, B, 2 * D), _F32),
            pltpu.VMEM((Dc // _LANES, (H + 1) * B, _LANES), _F32),
            pltpu.VMEM((Dc // _LANES, (B + 1) * H, _LANES), _F32),
            pltpu.VMEM((H, B, D), _F32),
            pltpu.SemaphoreType.DMA((n_sem,)),
            pltpu.SemaphoreType.DMA((B,)),
        ],
        compiler_params=pltpu.CompilerParams(
            vmem_limit_bytes=100 * 2**20,
            disable_semaphore_checks=True,
        ),
    )(*operands)
    return out.reshape(B, Sq, M)
```
